```python
import os as _os
_os.environ.setdefault("JAX_PLATFORMS", "cpu")
import jax
import jax.numpy as jnp

def _softmax(x, axis=-1):
    return jax.nn.softmax(x, axis=axis)
def _gelu(x):
    return jax.nn.gelu(x, approximate=True)
def _silu(x):
    return jax.nn.silu(x)
def _sigmoid(x):
    return jax.nn.sigmoid(x)
def _layernorm(x, axis=-1, eps=1e-5):
    m = jnp.mean(x, axis=axis, keepdims=True)
    v = jnp.var(x, axis=axis, keepdims=True)
    return (x - m) / jnp.sqrt(v + eps)
def _scatter_add(tgt, idx, src, axis=0):
    return tgt.at[idx].add(src)
def _segment_sum(src, seg, n):
    return jax.ops.segment_sum(src, seg, n)
class _Rng:
    def __init__(self, key):
        self._k = key
    def _next(self):
        self._k, sub = jax.random.split(self._k)
        return sub
    def normal(self, shape):
        return jax.random.normal(self._next(), shape, dtype=jnp.bfloat16)
    def randint(self, lo, hi, shape):
        return jax.random.randint(self._next(), shape, lo, hi, dtype=jnp.int32)
    def uniform(self, shape, lo=0.0, hi=1.0):
        return jax.random.uniform(self._next(), shape, jnp.bfloat16, lo, hi)
    def permutation(self, n):
        return jax.random.permutation(self._next(), n)


kernel_name = 'concat_heads__grouped_kv_mqa__sliding_block__prompt'

def setup_inputs():
    _rng = _Rng(jax.random.key(int.from_bytes(__import__("os").urandom(4), "little")))
    _w = (lambda a: (lambda t: t.astype(jnp.bfloat16) if jnp.issubdtype(t.dtype, jnp.floating) else t)(jnp.asarray(a)))
    def _A_setup():
        B, S, D, H = 1, 2048, 1024, 32
        Dh = D // H
        return {
            "x": _w((lambda *s: _rng.normal(s) * 0.05)(B, S, D)),
            "wq": _w((lambda *s: _rng.normal(s) * 1.6)(D, H * Dh)),
            "wk": _w((lambda *s: _rng.normal(s) * 1.6)(D, Dh)),
            "wv": _w((lambda *s: _rng.normal(s) * 0.1)(D, Dh)),
            "wo": _w((lambda *s: _rng.normal(s) * 0.1)(H * Dh, D)),
        }
    _A_in = _A_setup()

    def _B_setup():
        B, S, D = 1, 2048, 1024
        return {
            "x": _w((lambda *s: _rng.normal(s) * 0.2)(B, S, D)),
            "wqkv": _w((lambda *s: _rng.normal(s) * 0.2)(D, 3 * D)),
            "wo": _w((lambda *s: _rng.normal(s) * 0.05)(D, D)),
        }
    _B_in = _B_setup()

    return {
        "A_x": _A_in["x"],
        "A_wq": _A_in["wq"],
        "A_wk": _A_in["wk"],
        "A_wv": _A_in["wv"],
        "A_wo": _A_in["wo"],
        "B_x": _B_in["x"],
        "B_wqkv": _B_in["wqkv"],
        "B_wo": _B_in["wo"],
    }

def reference(A_x, A_wq, A_wk, A_wv, A_wo, B_x, B_wqkv, B_wo):
    def _A_ref(x, wq, wk, wv, wo):
        B, S, D = x.shape
        H = 32
        Dh = D // H
        q = (lambda x, *d: x.transpose(*d))((x @ wq).reshape(B, S, H, Dh), 0, 2, 1, 3)
        k = x @ wk
        v = x @ wv
        scores = jnp.einsum("bhqd,bkd->bhqk", q, k) * (Dh ** -0.5)
        p = _softmax(scores, axis=-1)
        o = jnp.einsum("bhqk,bkd->bhqd", p, v)
        return (lambda x, *d: x.transpose(*d))(o, 0, 2, 1, 3).reshape(B, S, H * Dh) @ wo

    def _B_ref(x, wqkv, wo):
        B, S, D = x.shape
        H = 32; Dh = D // H; W = 256
        qkv = (lambda x, *d: x.transpose(*d))((x @ wqkv).reshape(B, S, 3, H, Dh), 2, 0, 3, 1, 4)
        q, k, v = qkv[0], qkv[1], qkv[2]
        scores = jnp.einsum("bhqd,bhkd->bhqk", q, k) * (Dh ** -0.5)
        idx = jnp.arange(S)
        mask = (idx[:, None] - idx[None, :] >= 0) & (idx[:, None] - idx[None, :] < W)
        scores = jnp.where(mask[None, None], scores, -1e9)
        p = _softmax(scores, axis=-1)
        o = jnp.einsum("bhqk,bhkd->bhqd", p, v)
        return (lambda x, *d: x.transpose(*d))(o, 0, 2, 1, 3).reshape(B, S, D) @ wo

    a = _A_ref(A_x, A_wq, A_wk, A_wv, A_wo)
    b = _B_ref(B_x, B_wqkv, B_wo)
    return jnp.concatenate([a, b], axis=-1)
```

```python
import functools
import jax
import jax.numpy as jnp
from jax import lax
import jax.experimental.pallas as pl
import jax.experimental.pallas.tpu as pltpu

S = 2048
D = 1024
H = 32
DH = 32
W = 256
BQ = 128
NSTEP = S // BQ
KWIN = W + BQ
LOG2E = 1.4426950408889634
QSCALE = (DH ** -0.5) * LOG2E
NEG = -1e9 * LOG2E
_NT = (((1,), (1,)), ((), ()))


def _kernel(ax_ref, awq_ref, awk_ref, awv_ref, awo_ref, bx_ref, bwqkv_ref, bwo_ref,
            out_ref,
            awqT, ka, vaT, bwqT, bwvT, kwin, vTwin, qT, oT):
    i = pl.program_id(0)
    f32 = jnp.float32
    bf16 = jnp.bfloat16

    @pl.when(i == 0)
    def _init():
        awqT[...] = awq_ref[...].T
        bwqT[...] = bwqkv_ref[:, 0:D].T
        bwvT[...] = bwqkv_ref[:, 2 * D:3 * D].T
        x = ax_ref[...]
        ka[...] = jnp.dot(x, awk_ref[...], preferred_element_type=f32).astype(bf16)
        v = jnp.dot(x, awv_ref[...], preferred_element_type=f32)
        vaT[...] = v.T.astype(bf16)
        kwin[...] = jnp.zeros(kwin.shape, bf16)
        vTwin[...] = jnp.zeros(vTwin.shape, bf16)

    xa = ax_ref[pl.ds(pl.multiple_of(i * BQ, BQ), BQ), :]
    qT[...] = (lax.dot_general(awqT[...], xa, _NT, preferred_element_type=f32) * QSCALE).astype(bf16)

    def head_a(h, carry):
        r = pl.multiple_of(h * DH, DH)
        sT = jnp.dot(ka[...], qT[pl.ds(r, DH), :], preferred_element_type=f32)
        m = jnp.max(sT, axis=0, keepdims=True)
        p = jnp.exp2(sT - m)
        l = jnp.sum(p, axis=0, keepdims=True)
        o = jnp.dot(vaT[...], p.astype(bf16), preferred_element_type=f32)
        oT[pl.ds(r, DH), :] = (o / l).astype(bf16)
        return carry

    lax.fori_loop(0, H, head_a, 0, unroll=2)
    out_ref[:, 0:D] = jnp.dot(oT[...].T, awo_ref[...], preferred_element_type=f32).astype(out_ref.dtype)

    xb = bx_ref[...]
    qT[...] = (lax.dot_general(bwqT[...], xb, _NT, preferred_element_type=f32) * QSCALE).astype(bf16)
    kb = jnp.dot(xb, bwqkv_ref[:, D:2 * D], preferred_element_type=f32).astype(bf16)
    vbT = lax.dot_general(bwvT[...], xb, _NT, preferred_element_type=f32).astype(bf16)
    for g in range(H // 4):
        kwin[g, 0:W, :] = kwin[g, BQ:KWIN, :]
        kwin[g, W:KWIN, :] = kb[:, 128 * g:128 * (g + 1)]
    vTwin[:, 0:W] = vTwin[:, BQ:KWIN]
    vTwin[:, W:KWIN] = vbT

    kk = lax.broadcasted_iota(jnp.int32, (KWIN, BQ), 0)
    qq = lax.broadcasted_iota(jnp.int32, (KWIN, BQ), 1)
    diff = qq + W - kk
    valid = (diff >= 0) & (diff < W) & (kk + (i * BQ - W) >= 0)
    row = lax.broadcasted_iota(jnp.int32, (128, BQ), 0)

    def group_b(g, carry):
        r4 = pl.multiple_of(g * 128, 128)
        q4 = qT[pl.ds(r4, 128), :]
        k4 = kwin[g]
        for j in range(4):
            qm = jnp.where((row >= DH * j) & (row < DH * (j + 1)), q4, jnp.zeros_like(q4))
            sT = jnp.dot(k4, qm, preferred_element_type=f32)
            sT = jnp.where(valid, sT, NEG)
            m = jnp.max(sT, axis=0, keepdims=True)
            p = jnp.exp2(sT - m)
            l = jnp.sum(p, axis=0, keepdims=True)
            r = pl.multiple_of(g * 128 + DH * j, DH)
            o = jnp.dot(vTwin[pl.ds(r, DH), :], p.astype(bf16), preferred_element_type=f32)
            oT[pl.ds(r, DH), :] = (o / l).astype(bf16)
        return carry

    lax.fori_loop(0, H // 4, group_b, 0)
    out_ref[:, D:2 * D] = jnp.dot(oT[...].T, bwo_ref[...], preferred_element_type=f32).astype(out_ref.dtype)


@jax.jit
def pallas_concat_heads__grouped_kv_mqa__sliding_block__prompt_kernel(A_x, A_wq, A_wk, A_wv, A_wo, B_x, B_wqkv, B_wo):
    ax = A_x.reshape(S, D)
    bx = B_x.reshape(S, D)
    bf16 = jnp.bfloat16
    full = lambda shape: pl.BlockSpec(shape, lambda i: (0,) * len(shape))
    out = pl.pallas_call(
        _kernel,
        grid=(NSTEP,),
        in_specs=[
            full((S, D)), full((D, D)), full((D, DH)), full((D, DH)), full((D, D)),
            pl.BlockSpec((BQ, D), lambda i: (i, 0)),
            full((D, 3 * D)), full((D, D)),
        ],
        out_specs=pl.BlockSpec((BQ, 2 * D), lambda i: (i, 0)),
        out_shape=jax.ShapeDtypeStruct((S, 2 * D), bf16),
        scratch_shapes=[
            pltpu.VMEM((D, D), bf16),
            pltpu.VMEM((S, DH), bf16),
            pltpu.VMEM((DH, S), bf16),
            pltpu.VMEM((D, D), bf16),
            pltpu.VMEM((D, D), bf16),
            pltpu.VMEM((H // 4, KWIN, 128), bf16),
            pltpu.VMEM((D, KWIN), bf16),
            pltpu.VMEM((D, BQ), bf16),
            pltpu.VMEM((D, BQ), bf16),
        ],
        compiler_params=pltpu.CompilerParams(
            dimension_semantics=("arbitrary",),
            vmem_limit_bytes=100 * 1024 * 1024),
    )(ax, A_wq, A_wk, A_wv, A_wo, bx, B_wqkv, B_wo)
    return out.reshape(1, S, 2 * D)
```

```python
import functools
import jax
import jax.numpy as jnp
from jax import lax
import jax.experimental.pallas as pl
import jax.experimental.pallas.tpu as pltpu

S = 2048
D = 1024
H = 32
DH = 32
W = 256
BQ = 1024
NSTEP = S // BQ
SB = 128
NSB = BQ // SB
KSB = W + SB
KWIN = W + BQ
CK = 128
TQ = 128
NC = S // CK
NT = BQ // TQ
LAG = 8
PC = 256
OC = 256
LOG2E = 1.4426950408889634
QSCALE = (DH ** -0.5) * LOG2E
NEG = -1e9 * LOG2E
_NT = (((1,), (1,)), ((), ()))
UNITS = [(c, t) for c in range(NC) for t in range(NT)]
NU = len(UNITS)


def _kernel(ax_hbm, awq_hbm, awk_ref, awv_ref, awo_hbm, bx_ref, bwqkv_hbm, bwo_hbm,
            out_hbm,
            ax_ref, awq_ref, awo_ref, bwqkv_ref, bwo_ref, sems, obuf, osems,
            awqT, ka, vaT, bwqT, bwvT, kwin, vTwin, qT, oT, biasb, scar):
    i = pl.program_id(0)
    f32 = jnp.float32
    bf16 = jnp.bfloat16

    cp_awq = pltpu.make_async_copy(awq_hbm, awq_ref, sems.at[0])
    cp_ax0 = pltpu.make_async_copy(ax_hbm.at[pl.ds(0, BQ), :], ax_ref.at[pl.ds(0, BQ), :], sems.at[1])
    cp_ax1 = pltpu.make_async_copy(ax_hbm.at[pl.ds(BQ, S - BQ), :], ax_ref.at[pl.ds(BQ, S - BQ), :], sems.at[2])
    cp_awo = pltpu.make_async_copy(awo_hbm, awo_ref, sems.at[3])
    cp_bw = pltpu.make_async_copy(bwqkv_hbm, bwqkv_ref, sems.at[4])
    cp_bwo = pltpu.make_async_copy(bwo_hbm, bwo_ref, sems.at[5])

    def out_copy(c, half):
        r = pl.multiple_of(c * OC, OC)
        return pltpu.make_async_copy(
            obuf.at[pl.ds(r, OC), pl.ds(half * D, D)],
            out_hbm.at[pl.ds(i * BQ + r, OC), pl.ds(half * D, D)],
            osems.at[half * (BQ // OC) + c])

    @pl.when(i == 0)
    def _init():
        cp_awq.start()
        kwin[:, 0:W, :] = jnp.zeros((H // 4, W, 128), bf16)
        vTwin[:, 0:W] = jnp.zeros((D, W), bf16)
        cp_awq.wait()
        cp_ax0.start()
        awqT[...] = awq_ref[...].T
        cp_ax0.wait()
        cp_ax1.start()

    def qproj_a(c, carry):
        r = pl.multiple_of(c * PC, PC)
        xa = ax_ref[pl.ds(pl.multiple_of(i * BQ, BQ), BQ), :]
        qT[pl.ds(r, PC), :] = (lax.dot_general(awqT[pl.ds(r, PC), :], xa, _NT,
                                               preferred_element_type=f32) * QSCALE).astype(bf16)
        return carry

    lax.fori_loop(0, D // PC, qproj_a, 0)

    @pl.when(i == 0)
    def _init_kv():
        cp_ax1.wait()
        cp_awo.start()
        cp_bw.start()
        cp_bwo.start()
        wkvT = jnp.concatenate([awk_ref[...], awv_ref[...]], axis=0)
        kvT = lax.dot_general(wkvT, ax_ref[...], _NT, preferred_element_type=f32)
        ka[...] = kvT[0:DH, :].T.astype(bf16)
        vaT[...] = kvT[DH:2 * DH, :].astype(bf16)

    def pv_unit(u, s, st):
        c, t = UNITS[u]
        cm = jnp.max(s, axis=0, keepdims=True)
        vt = vaT[:, c * CK:(c + 1) * CK]
        if st[t] is None:
            p = jnp.exp2(s - cm)
            l8 = jnp.sum(p.reshape(CK // 8, 8, TQ), axis=0)
            acc = jnp.dot(vt, p.astype(bf16), preferred_element_type=f32)
            st[t] = (cm, l8, acc)
        else:
            m, l8, acc = st[t]
            mn = jnp.maximum(m, cm)
            alpha = jnp.exp2(m - mn)
            p = jnp.exp2(s - mn)
            l8 = l8 * alpha + jnp.sum(p.reshape(CK // 8, 8, TQ), axis=0)
            acc = acc * alpha + jnp.dot(vt, p.astype(bf16), preferred_element_type=f32)
            st[t] = (mn, l8, acc)

    def fin(h, t, st):
        m, l8, acc = st[t]
        l = jnp.sum(l8, axis=0, keepdims=True)
        oT[pl.ds(pl.multiple_of(h * DH, DH), DH), t * TQ:(t + 1) * TQ] = (acc / l).astype(bf16)

    def body(h, prev, do_qk=True):
        if do_qk:
            r = pl.multiple_of(h * DH, DH)
            qs = [qT[pl.ds(r, DH), t * TQ:(t + 1) * TQ] for t in range(NT)]
        sc = {}
        pend = []
        st = [None] * NT
        pst = list(prev) if prev is not None else None
        for u in range(NU if do_qk else LAG):
            if do_qk:
                c, t = UNITS[u]
                sv = jnp.dot(ka[c * CK:(c + 1) * CK, :], qs[t], preferred_element_type=f32)
                if u >= NU - LAG:
                    pend.append((u - (NU - LAG), sv))
                else:
                    sc[u] = sv
            if u < LAG:
                if pst is not None:
                    pu = NU - LAG + u
                    pv_unit(pu, scar[u], pst)
                    if pu >= NU - NT:
                        fin(h - 1, UNITS[pu][1], pst)
            else:
                pv_unit(u - LAG, sc.pop(u - LAG), st)
        if do_qk:
            for k, sv in pend:
                scar[k] = sv
            return tuple(st)

    carry = body(0, None)
    carry = lax.fori_loop(1, H, lambda h, c: body(h, c), carry)
    body(H, carry, do_qk=False)

    @pl.when(i == 0)
    def _():
        cp_awo.wait()

    def oproj_a(c, carry):
        r = pl.multiple_of(c * OC, OC)
        obuf[pl.ds(r, OC), 0:D] = jnp.dot(oT[:, pl.ds(r, OC)].T, awo_ref[...],
                                          preferred_element_type=f32).astype(bf16)
        out_copy(c, 0).start()
        return carry

    lax.fori_loop(0, BQ // OC, oproj_a, 0)

    @pl.when(i == 0)
    def _():
        cp_bw.wait()
        bwqT[...] = bwqkv_ref[:, 0:D].T
        bwvT[...] = bwqkv_ref[:, 2 * D:3 * D].T

    @pl.when(i > 0)
    def _():
        for g in range(H // 4):
            kwin[g, 0:W, :] = kwin[g, BQ:KWIN, :]
        vTwin[:, 0:W] = vTwin[:, BQ:KWIN]

    def proj_b(c, carry):
        r = pl.multiple_of(c * PC, PC)
        xb = bx_ref[...]
        qT[pl.ds(r, PC), :] = (lax.dot_general(bwqT[pl.ds(r, PC), :], xb, _NT,
                                               preferred_element_type=f32) * QSCALE).astype(bf16)
        vTwin[pl.ds(r, PC), W:KWIN] = lax.dot_general(bwvT[pl.ds(r, PC), :], xb, _NT,
                                                      preferred_element_type=f32).astype(bf16)
        r2 = pl.multiple_of(c * OC, OC)
        kb = jnp.dot(bx_ref[pl.ds(r2, OC), :], bwqkv_ref[:, D:2 * D], preferred_element_type=f32).astype(bf16)
        for g in range(H // 4):
            kwin[g, pl.ds(W + r2, OC), :] = kb[:, 128 * g:128 * (g + 1)]
        return carry

    lax.fori_loop(0, D // PC, proj_b, 0)

    kk = lax.broadcasted_iota(jnp.int32, (KSB, SB), 0)
    qq = lax.broadcasted_iota(jnp.int32, (KSB, SB), 1)
    diff = qq + W - kk
    band = (diff >= 0) & (diff < W)
    valid = [band & (kk + (i * BQ + b * SB - W) >= 0) if b * SB < W else band for b in range(NSB)]
    row = lax.broadcasted_iota(jnp.int32, (128, SB), 0)
    for b in range(3):
        biasb[b] = jnp.where(valid[b], 0.0, NEG).astype(f32)

    def group_b(g, carry):
        r4 = pl.multiple_of(g * 128, 128)

        def make_qm(b):
            q4 = qT[pl.ds(r4, 128), b * SB:(b + 1) * SB]
            z = jnp.zeros_like(q4)
            return jnp.concatenate(
                [jnp.where((row >= DH * j) & (row < DH * (j + 1)), q4, z) for j in range(4)], axis=1)

        def qk_piece(b, qm, kb_):
            k4 = kwin[g, (b + kb_) * SB:(b + kb_ + 1) * SB, :]
            s = jnp.dot(k4, qm, preferred_element_type=f32)
            if b < 2 or kb_ != 1:
                bias = biasb[min(b, 2), kb_ * SB:(kb_ + 1) * SB, :]
                s = s + jnp.concatenate([bias] * 4, axis=1)
            cm = jnp.max(s.reshape(SB // 8, 8, 4 * SB), axis=0)
            return s, cm

        def pv_piece(b, kb_, s, m, l8, accs):
            p = jnp.exp2(s - m)
            ps = jnp.sum(p.reshape(SB // 8, 8, 4 * SB), axis=0)
            l8 = ps if l8 is None else l8 + ps
            pb = p.astype(bf16)
            new = []
            for j in range(4):
                r = pl.multiple_of(g * 128 + DH * j, DH)
                o = jnp.dot(vTwin[pl.ds(r, DH), (b + kb_) * SB:(b + kb_ + 1) * SB],
                            pb[:, j * SB:(j + 1) * SB], preferred_element_type=f32)
                new.append(o if accs is None else accs[j] + o)
            return l8, new

        ILAG = 1
        done = {}
        prev_cm = None
        for t in range(NSB + ILAG):
            nxt_s = []
            mx = None
            l8 = None
            accs = None
            cur = done.pop(t - ILAG, None)
            if t < NSB:
                qm = make_qm(t)
            for kb_ in range(3):
                if t < NSB:
                    s, cm = qk_piece(t, qm, kb_)
                    nxt_s.append(s)
                    mx = cm if mx is None else jnp.maximum(mx, cm)
                if cur is not None:
                    mm = cur[2]
                    if t < NSB and prev_cm is not None:
                        d = prev_cm[0:1, :]
                        mm = jnp.where(d > 3e38, d, mm)
                    l8, accs = pv_piece(cur[0], kb_, cur[1][kb_], mm, l8, accs)
                if t < NSB:
                    prev_cm = cm
            if cur is not None:
                b = cur[0]
                l = jnp.sum(l8, axis=0, keepdims=True)
                for j in range(4):
                    r = pl.multiple_of(g * 128 + DH * j, DH)
                    oT[pl.ds(r, DH), b * SB:(b + 1) * SB] = (accs[j] / l[:, j * SB:(j + 1) * SB]).astype(bf16)
            if t < NSB:
                done[t] = (t, nxt_s, jnp.max(mx, axis=0, keepdims=True))
        return carry

    lax.fori_loop(0, H // 4, group_b, 0)

    @pl.when(i == 0)
    def _():
        cp_bwo.wait()

    def oproj_b(c, carry):
        r = pl.multiple_of(c * OC, OC)
        obuf[pl.ds(r, OC), D:2 * D] = jnp.dot(oT[:, pl.ds(r, OC)].T, bwo_ref[...],
                                              preferred_element_type=f32).astype(bf16)
        out_copy(c, 1).start()
        return carry

    lax.fori_loop(0, BQ // OC, oproj_b, 0)
    for half in range(2):
        for c in range(BQ // OC):
            out_copy(c, half).wait()


@jax.jit
def pallas_concat_heads__grouped_kv_mqa__sliding_block__prompt_kernel(A_x, A_wq, A_wk, A_wv, A_wo, B_x, B_wqkv, B_wo):
    ax = A_x.reshape(S, D)
    bx = B_x.reshape(S, D)
    bf16 = jnp.bfloat16
    full = lambda shape: pl.BlockSpec(shape, lambda i: (0,) * len(shape))
    hbm = pl.BlockSpec(memory_space=pl.ANY)
    out = pl.pallas_call(
        _kernel,
        grid=(NSTEP,),
        in_specs=[
            hbm, hbm, full((DH, D)), full((DH, D)), hbm,
            pl.BlockSpec((BQ, D), lambda i: (i, 0)),
            hbm, hbm,
        ],
        out_specs=hbm,
        out_shape=jax.ShapeDtypeStruct((S, 2 * D), bf16),
        scratch_shapes=[
            pltpu.VMEM((S, D), bf16),
            pltpu.VMEM((D, D), bf16),
            pltpu.VMEM((D, D), bf16),
            pltpu.VMEM((D, 3 * D), bf16),
            pltpu.VMEM((D, D), bf16),
            pltpu.SemaphoreType.DMA((6,)),
            pltpu.VMEM((BQ, 2 * D), bf16),
            pltpu.SemaphoreType.DMA((2 * (BQ // OC),)),
            pltpu.VMEM((D, D), bf16),
            pltpu.VMEM((S, DH), bf16),
            pltpu.VMEM((DH, S), bf16),
            pltpu.VMEM((D, D), bf16),
            pltpu.VMEM((D, D), bf16),
            pltpu.VMEM((H // 4, KWIN, 128), bf16),
            pltpu.VMEM((D, KWIN), bf16),
            pltpu.VMEM((D, BQ), bf16),
            pltpu.VMEM((D, BQ), bf16),
            pltpu.VMEM((3, KSB, SB), jnp.float32),
            pltpu.VMEM((LAG, CK, TQ), jnp.float32),
        ],
        compiler_params=pltpu.CompilerParams(
            dimension_semantics=("arbitrary",),
            vmem_limit_bytes=100 * 1024 * 1024),
    )(ax, A_wq, A_wk.T, A_wv.T, A_wo, bx, B_wqkv, B_wo)
    return out.reshape(1, S, 2 * D)
```

```python
import functools
import jax
import jax.numpy as jnp
from jax import lax
import jax.experimental.pallas as pl
import jax.experimental.pallas.tpu as pltpu

S = 2048
D = 1024
H = 32
DH = 32
W = 256
BQ = 1024
NSTEP = S // BQ
SB = 128
NSB = BQ // SB
KSB = W + SB
KWIN = W + BQ
CK = 128
TQ = 128
NC = S // CK
NT = BQ // TQ
LAG = 8
PC = 256
OC = 256
LOG2E = 1.4426950408889634
QSCALE = (DH ** -0.5) * LOG2E
NEG = -1e9 * LOG2E
_NT = (((1,), (1,)), ((), ()))
UNITS = [(c, t) for c in range(NC) for t in range(NT)]
NU = len(UNITS)


def _kernel(ax_hbm, awq_hbm, awk_ref, awv_ref, awo_hbm, bx_ref, bwqkv_hbm, bwo_hbm,
            out_hbm,
            ax_ref, awq_ref, awo_ref, bwqkv_ref, bwo_ref, sems, obuf, osems,
            awqT, ka, vaT, bwqT, bwvT, kwin, vTwin, qT, oT, biasb, scar):
    i = pl.program_id(0)
    f32 = jnp.float32
    bf16 = jnp.bfloat16

    cp_awq = pltpu.make_async_copy(awq_hbm, awq_ref, sems.at[0])
    cp_ax0 = pltpu.make_async_copy(ax_hbm.at[pl.ds(0, BQ), :], ax_ref.at[pl.ds(0, BQ), :], sems.at[1])
    cp_ax1 = pltpu.make_async_copy(ax_hbm.at[pl.ds(BQ, S - BQ), :], ax_ref.at[pl.ds(BQ, S - BQ), :], sems.at[2])
    cp_awo = pltpu.make_async_copy(awo_hbm, awo_ref, sems.at[3])
    cp_bw = pltpu.make_async_copy(bwqkv_hbm, bwqkv_ref, sems.at[4])
    cp_bwo = pltpu.make_async_copy(bwo_hbm, bwo_ref, sems.at[5])

    def out_copy(c, half):
        r = pl.multiple_of(c * OC, OC)
        return pltpu.make_async_copy(
            obuf.at[pl.ds(r, OC), pl.ds(half * D, D)],
            out_hbm.at[pl.ds(i * BQ + r, OC), pl.ds(half * D, D)],
            osems.at[half * (BQ // OC) + c])

    @pl.when(i == 0)
    def _init():
        cp_awq.start()
        kwin[:, 0:W, :] = jnp.zeros((H // 4, W, 128), bf16)
        vTwin[:, 0:W] = jnp.zeros((D, W), bf16)
        cp_awq.wait()
        cp_ax0.start()
        awqT[...] = awq_ref[...].T
        cp_ax0.wait()
        cp_ax1.start()

    def qproj_a(c, carry):
        r = pl.multiple_of(c * PC, PC)
        xa = ax_ref[pl.ds(pl.multiple_of(i * BQ, BQ), BQ), :]
        qT[pl.ds(r, PC), :] = (lax.dot_general(awqT[pl.ds(r, PC), :], xa, _NT,
                                               preferred_element_type=f32) * QSCALE).astype(bf16)
        return carry

    lax.fori_loop(0, D // PC, qproj_a, 0)

    @pl.when(i == 0)
    def _init_kv():
        cp_ax1.wait()
        cp_awo.start()
        cp_bw.start()
        cp_bwo.start()
        wkvT = jnp.concatenate([awk_ref[...], awv_ref[...]], axis=0)
        kvT = lax.dot_general(wkvT, ax_ref[...], _NT, preferred_element_type=f32)
        ka[...] = kvT[0:DH, :].T.astype(bf16)
        vaT[...] = kvT[DH:2 * DH, :].astype(bf16)

    def pv_unit(u, s, st):
        c, t = UNITS[u]
        cm = jnp.max(s, axis=0, keepdims=True)
        vt = vaT[:, c * CK:(c + 1) * CK]
        if st[t] is None:
            p = jnp.exp2(s - cm)
            l8 = jnp.sum(p.reshape(CK // 8, 8, TQ), axis=0)
            acc = jnp.dot(vt, p.astype(bf16), preferred_element_type=f32)
            st[t] = (cm, l8, acc)
        else:
            m, l8, acc = st[t]
            mn = jnp.maximum(m, cm)
            alpha = jnp.exp2(m - mn)
            p = jnp.exp2(s - mn)
            l8 = l8 * alpha + jnp.sum(p.reshape(CK // 8, 8, TQ), axis=0)
            acc = acc * alpha + jnp.dot(vt, p.astype(bf16), preferred_element_type=f32)
            st[t] = (mn, l8, acc)

    def fin(h, t, st):
        m, l8, acc = st[t]
        l = jnp.sum(l8, axis=0, keepdims=True)
        hh = jnp.maximum(h, 0)
        oT[pl.ds(pl.multiple_of(hh * DH, DH), DH), t * TQ:(t + 1) * TQ] = (acc / l).astype(bf16)

    def body(h, prev, do_qk=True):
        if do_qk:
            r = pl.multiple_of(h * DH, DH)
            qs = [qT[pl.ds(r, DH), t * TQ:(t + 1) * TQ] for t in range(NT)]
        sc = {}
        pend = []
        st = [None] * NT
        pst = list(prev) if prev is not None else None
        for u in range(NU if do_qk else LAG):
            if do_qk:
                c, t = UNITS[u]
                sv = jnp.dot(ka[c * CK:(c + 1) * CK, :], qs[t], preferred_element_type=f32)
                if u >= NU - LAG:
                    pend.append((u - (NU - LAG), sv))
                else:
                    sc[u] = sv
            if u < LAG:
                if pst is not None:
                    pu = NU - LAG + u
                    pv_unit(pu, scar[u], pst)
                    if pu >= NU - NT:
                        fin(h - 1, UNITS[pu][1], pst)
            else:
                pv_unit(u - LAG, sc.pop(u - LAG), st)
        if do_qk:
            for k, sv in pend:
                scar[k] = sv
            return tuple(st)

    scar[...] = jnp.zeros(scar.shape, f32)
    dummy = tuple((jnp.zeros((1, TQ), f32), jnp.ones((8, TQ), f32), jnp.zeros((DH, TQ), f32))
                  for _ in range(NT))

    def pair(j, c):
        for k in range(4):
            c = body(4 * j + k, c)
        return c

    carry = lax.fori_loop(0, H // 4, pair, dummy)
    body(H, carry, do_qk=False)

    @pl.when(i == 0)
    def _():
        cp_awo.wait()

    def oproj_a(c, carry):
        r = pl.multiple_of(c * OC, OC)
        obuf[pl.ds(r, OC), 0:D] = jnp.dot(oT[:, pl.ds(r, OC)].T, awo_ref[...],
                                          preferred_element_type=f32).astype(bf16)
        out_copy(c, 0).start()
        return carry

    lax.fori_loop(0, BQ // OC, oproj_a, 0)

    @pl.when(i == 0)
    def _():
        cp_bw.wait()
        bwqT[...] = bwqkv_ref[:, 0:D].T
        bwvT[...] = bwqkv_ref[:, 2 * D:3 * D].T

    @pl.when(i > 0)
    def _():
        for g in range(H // 4):
            kwin[g, 0:W, :] = kwin[g, BQ:KWIN, :]
        vTwin[:, 0:W] = vTwin[:, BQ:KWIN]

    def proj_b(c, carry):
        r = pl.multiple_of(c * PC, PC)
        xb = bx_ref[...]
        qT[pl.ds(r, PC), :] = (lax.dot_general(bwqT[pl.ds(r, PC), :], xb, _NT,
                                               preferred_element_type=f32) * QSCALE).astype(bf16)
        vTwin[pl.ds(r, PC), W:KWIN] = lax.dot_general(bwvT[pl.ds(r, PC), :], xb, _NT,
                                                      preferred_element_type=f32).astype(bf16)
        r2 = pl.multiple_of(c * OC, OC)
        kb = jnp.dot(bx_ref[pl.ds(r2, OC), :], bwqkv_ref[:, D:2 * D], preferred_element_type=f32).astype(bf16)
        for g in range(H // 4):
            kwin[g, pl.ds(W + r2, OC), :] = kb[:, 128 * g:128 * (g + 1)]
        return carry

    lax.fori_loop(0, D // PC, proj_b, 0)

    kk = lax.broadcasted_iota(jnp.int32, (KSB, SB), 0)
    qq = lax.broadcasted_iota(jnp.int32, (KSB, SB), 1)
    diff = qq + W - kk
    band = (diff >= 0) & (diff < W)
    valid = [band & (kk + (i * BQ + b * SB - W) >= 0) if b * SB < W else band for b in range(NSB)]
    row = lax.broadcasted_iota(jnp.int32, (128, SB), 0)
    for b in range(3):
        biasb[b] = jnp.where(valid[b], 0.0, NEG).astype(f32)

    GB = 2

    def group_b(gi, carry):
        def make_qm(g, b):
            r4 = pl.multiple_of(g * 128, 128)
            q4 = qT[pl.ds(r4, 128), b * SB:(b + 1) * SB]
            z = jnp.zeros_like(q4)
            return jnp.concatenate(
                [jnp.where((row >= DH * j) & (row < DH * (j + 1)), q4, z) for j in range(4)], axis=1)

        def qk_piece(g, b, qm, kb_):
            k4 = kwin[g, (b + kb_) * SB:(b + kb_ + 1) * SB, :]
            s = jnp.dot(k4, qm, preferred_element_type=f32)
            if b < 2 or kb_ != 1:
                bias = biasb[min(b, 2), kb_ * SB:(kb_ + 1) * SB, :]
                s = s + jnp.concatenate([bias] * 4, axis=1)
            cm = jnp.max(s.reshape(SB // 8, 8, 4 * SB), axis=0)
            return s, cm

        def pv_piece(g, b, kb_, s, m, l8, accs):
            p = jnp.exp2(s - m)
            ps = jnp.sum(p.reshape(SB // 8, 8, 4 * SB), axis=0)
            l8 = ps if l8 is None else l8 + ps
            pb = p.astype(bf16)
            new = []
            for j in range(4):
                r = pl.multiple_of(g * 128 + DH * j, DH)
                o = jnp.dot(vTwin[pl.ds(r, DH), (b + kb_) * SB:(b + kb_ + 1) * SB],
                            pb[:, j * SB:(j + 1) * SB], preferred_element_type=f32)
                new.append(o if accs is None else accs[j] + o)
            return l8, new

        items = [(gi * GB + gg, b) for gg in range(GB) for b in range(NSB)]
        n = len(items)
        cur = None
        prev_cm = None
        for t in range(n + 1):
            nxt_s = []
            mx = None
            l8 = None
            accs = None
            if t < n:
                g, b = items[t]
                qm = make_qm(g, b)
            for kb_ in range(3):
                if t < n:
                    s, cm = qk_piece(g, b, qm, kb_)
                    nxt_s.append(s)
                    mx = cm if mx is None else jnp.maximum(mx, cm)
                if cur is not None:
                    mm = cur[3]
                    if t < n and prev_cm is not None:
                        mm = jnp.maximum(mm, jnp.minimum(prev_cm[0:1, :], mm))
                    l8, accs = pv_piece(cur[0], cur[1], kb_, cur[2][kb_], mm, l8, accs)
                if t < n:
                    prev_cm = cm
            if cur is not None:
                cg, cb = cur[0], cur[1]
                l = jnp.sum(l8, axis=0, keepdims=True)
                for j in range(4):
                    r = pl.multiple_of(cg * 128 + DH * j, DH)
                    oT[pl.ds(r, DH), cb * SB:(cb + 1) * SB] = (accs[j] / l[:, j * SB:(j + 1) * SB]).astype(bf16)
            cur = (g, b, nxt_s, jnp.max(mx, axis=0, keepdims=True)) if t < n else None
        return carry

    lax.fori_loop(0, H // 4 // GB, group_b, 0)

    @pl.when(i == 0)
    def _():
        cp_bwo.wait()

    def oproj_b(c, carry):
        r = pl.multiple_of(c * OC, OC)
        obuf[pl.ds(r, OC), D:2 * D] = jnp.dot(oT[:, pl.ds(r, OC)].T, bwo_ref[...],
                                              preferred_element_type=f32).astype(bf16)
        out_copy(c, 1).start()
        return carry

    lax.fori_loop(0, BQ // OC, oproj_b, 0)
    for half in range(2):
        for c in range(BQ // OC):
            out_copy(c, half).wait()


@jax.jit
def pallas_concat_heads__grouped_kv_mqa__sliding_block__prompt_kernel(A_x, A_wq, A_wk, A_wv, A_wo, B_x, B_wqkv, B_wo):
    ax = A_x.reshape(S, D)
    bx = B_x.reshape(S, D)
    bf16 = jnp.bfloat16
    full = lambda shape: pl.BlockSpec(shape, lambda i: (0,) * len(shape))
    hbm = pl.BlockSpec(memory_space=pl.ANY)
    out = pl.pallas_call(
        _kernel,
        grid=(NSTEP,),
        in_specs=[
            hbm, hbm, full((DH, D)), full((DH, D)), hbm,
            pl.BlockSpec((BQ, D), lambda i: (i, 0)),
            hbm, hbm,
        ],
        out_specs=hbm,
        out_shape=jax.ShapeDtypeStruct((S, 2 * D), bf16),
        scratch_shapes=[
            pltpu.VMEM((S, D), bf16),
            pltpu.VMEM((D, D), bf16),
            pltpu.VMEM((D, D), bf16),
            pltpu.VMEM((D, 3 * D), bf16),
            pltpu.VMEM((D, D), bf16),
            pltpu.SemaphoreType.DMA((6,)),
            pltpu.VMEM((BQ, 2 * D), bf16),
            pltpu.SemaphoreType.DMA((2 * (BQ // OC),)),
            pltpu.VMEM((D, D), bf16),
            pltpu.VMEM((S, DH), bf16),
            pltpu.VMEM((DH, S), bf16),
            pltpu.VMEM((D, D), bf16),
            pltpu.VMEM((D, D), bf16),
            pltpu.VMEM((H // 4, KWIN, 128), bf16),
            pltpu.VMEM((D, KWIN), bf16),
            pltpu.VMEM((D, BQ), bf16),
            pltpu.VMEM((D, BQ), bf16),
            pltpu.VMEM((3, KSB, SB), jnp.float32),
            pltpu.VMEM((LAG, CK, TQ), jnp.float32),
        ],
        compiler_params=pltpu.CompilerParams(
            dimension_semantics=("arbitrary",),
            vmem_limit_bytes=100 * 1024 * 1024),
    )(ax, A_wq, A_wk.T, A_wv.T, A_wo, bx, B_wqkv, B_wo)
    return out.reshape(1, S, 2 * D)
```
